```python
import os as _os
_os.environ.setdefault("JAX_PLATFORMS", "cpu")
import jax
import jax.numpy as jnp

def _softmax(x, axis=-1):
    return jax.nn.softmax(x, axis=axis)
def _gelu(x):
    return jax.nn.gelu(x, approximate=True)
def _silu(x):
    return jax.nn.silu(x)
def _sigmoid(x):
    return jax.nn.sigmoid(x)
def _layernorm(x, axis=-1, eps=1e-5):
    m = jnp.mean(x, axis=axis, keepdims=True)
    v = jnp.var(x, axis=axis, keepdims=True)
    return (x - m) / jnp.sqrt(v + eps)
def _scatter_add(tgt, idx, src, axis=0):
    return tgt.at[idx].add(src)
def _segment_sum(src, seg, n):
    return jax.ops.segment_sum(src, seg, n)
class _Rng:
    def __init__(self, key):
        self._k = key
    def _next(self):
        self._k, sub = jax.random.split(self._k)
        return sub
    def normal(self, shape):
        return jax.random.normal(self._next(), shape, dtype=jnp.bfloat16)
    def randint(self, lo, hi, shape):
        return jax.random.randint(self._next(), shape, lo, hi, dtype=jnp.int32)
    def uniform(self, shape, lo=0.0, hi=1.0):
        return jax.random.uniform(self._next(), shape, jnp.bfloat16, lo, hi)
    def permutation(self, n):
        return jax.random.permutation(self._next(), n)


kernel_name = 'interleave_layers__sliding_local_dilated__sliding_local_dilated__prompt'

def setup_inputs():
    _rng = _Rng(jax.random.key(int.from_bytes(__import__("os").urandom(4), "little")))
    _w = (lambda a: (lambda t: t.astype(jnp.bfloat16) if jnp.issubdtype(t.dtype, jnp.floating) else t)(jnp.asarray(a)))
    def _A_setup():
        B, S, D = 1, 2048, 1024
        return {
            "x": _w((lambda *s: _rng.normal(s) * 0.05)(B, S, D)),
            "wqkv": _w((lambda *s: _rng.normal(s) * 0.05)(D, 3 * D)),
            "wo": _w((lambda *s: _rng.normal(s) * 0.05)(D, D)),
        }
    _A_in = _A_setup()

    def _B_setup():
        B, S, D = 1, 2048, 1024
        return {
            "x": _w((lambda *s: _rng.normal(s) * 0.05)(B, S, D)),
            "wqkv": _w((lambda *s: _rng.normal(s) * 0.05)(D, 3 * D)),
            "wo": _w((lambda *s: _rng.normal(s) * 0.05)(D, D)),
        }
    _B_in = _B_setup()

    return {
        "A_x": _A_in["x"],
        "A_wqkv": _A_in["wqkv"],
        "A_wo": _A_in["wo"],
        "B_x": _B_in["x"],
        "B_wqkv": _B_in["wqkv"],
        "B_wo": _B_in["wo"],
    }

def reference(A_x, A_wqkv, A_wo, B_x, B_wqkv, B_wo):
    def _A_ref(x, wqkv, wo):
        B, S, D = x.shape
        H = 32; Dh = D // H
        W, dil = 8, 2
        qkv = (lambda x, *d: x.transpose(*d))((x @ wqkv).reshape(B, S, 3, H, Dh), 2, 0, 3, 1, 4)
        q, k, v = qkv[0], qkv[1], qkv[2]
        scale = Dh ** -0.5
        pos = jnp.arange(S)
        off = jnp.arange(W) * dil
        idx = pos[:, None] - off[None, :]
        mask = idx >= 0
        idx_c = jnp.where(mask, idx, 0).reshape(-1)
        kg = k[:, :, idx_c, :].reshape(B, H, S, W, Dh)
        vg = v[:, :, idx_c, :].reshape(B, H, S, W, Dh)
        logits = jnp.einsum("bhsd,bhswd->bhsw", q, kg) * scale
        logits = jnp.where(mask[None, None, :, :], logits, -1e9)
        attn = _softmax(logits, axis=-1)
        o = jnp.einsum("bhsw,bhswd->bhsd", attn, vg)
        return (lambda x, *d: x.transpose(*d))(o, 0, 2, 1, 3).reshape(B, S, D) @ wo

    def _B_ref(x, wqkv, wo):
        B, S, D = x.shape
        H = 32; Dh = D // H
        W, dil = 8, 2
        qkv = (lambda x, *d: x.transpose(*d))((x @ wqkv).reshape(B, S, 3, H, Dh), 2, 0, 3, 1, 4)
        q, k, v = qkv[0], qkv[1], qkv[2]
        scale = Dh ** -0.5
        pos = jnp.arange(S)
        off = jnp.arange(W) * dil
        idx = pos[:, None] - off[None, :]
        mask = idx >= 0
        idx_c = jnp.where(mask, idx, 0).reshape(-1)
        kg = k[:, :, idx_c, :].reshape(B, H, S, W, Dh)
        vg = v[:, :, idx_c, :].reshape(B, H, S, W, Dh)
        logits = jnp.einsum("bhsd,bhswd->bhsw", q, kg) * scale
        logits = jnp.where(mask[None, None, :, :], logits, -1e9)
        attn = _softmax(logits, axis=-1)
        o = jnp.einsum("bhsw,bhswd->bhsd", attn, vg)
        return (lambda x, *d: x.transpose(*d))(o, 0, 2, 1, 3).reshape(B, S, D) @ wo

    x = A_x
    x = x + _A_ref(_layernorm(x, axis=-1), A_wqkv, A_wo)
    x = x + _B_ref(_layernorm(x, axis=-1), B_wqkv, B_wo)
    x = x + _A_ref(_layernorm(x, axis=-1), A_wqkv, A_wo)
    x = x + _B_ref(_layernorm(x, axis=-1), B_wqkv, B_wo)
    return x
```

```python
import functools

import jax
import jax.numpy as jnp
from jax import lax
from jax.experimental import pallas as pl
from jax.experimental.pallas import tpu as pltpu

S, D, H, W, DIL = 2048, 1024, 32, 8, 2
DH = D // H
N_LAYERS = 4
LANES = 128
NJ = D // LANES
BM = 128
HB = BM // 2
NB = S // BM
T = N_LAYERS * NB
HALO = 16
CH = 16
KP = 256
NK = D // KP
GW = 4 * LANES
PADH = DH + 1
SCALE = DH ** -0.5
LOG2E = 1.4426950408889634
F32, BF16, U32, I32 = jnp.float32, jnp.bfloat16, jnp.uint32, jnp.int32

B_LEAD, B_BACK = 5, 3
N_LEAD, N_BACK = 6, 2
W_PER_PHASE, J_PER_PHASE = 4, 2
B_PHASES = (BM // CH) * ((CH // 8) * (W // W_PER_PHASE) + NJ // J_PER_PHASE)
WO_PHASES = 4

_NT = (((1,), (1,)), ((), ()))


def _pack(v):
    return pltpu.bitcast(v.astype(BF16), U32)


def _unpack(v):
    return pltpu.bitcast(v, BF16)


def _token(vals):
    parts = []
    for v in vals:
        v = v if v.dtype == U32 else pltpu.bitcast(v, U32)
        parts += [v[r:r + 8, c:c + LANES] for r in range(0, v.shape[0], 8) for c in range(0, v.shape[1], LANES)]
    return functools.reduce(jnp.bitwise_or, parts)


def _aligned(v, m):
    return v if isinstance(v, int) else pl.multiple_of(v, m)


def _drain(gen):
    for _ in gen:
        pass


def _kernel(x_hbm, wqa_hbm, woa_hbm, wqb_hbm, wob_hbm, out_hbm,
            xs0, xs1, xn0, xn1, ob0, ob1, q0, q1, k0, k1, v0, v1,
            wqT, wop, wq_raw, wo_raw, tbuf, odd, xsem, wsem):
    xs, xn, ob, qb, kb, vb = (xs0, xs1), (xn0, xn1), (ob0, ob1), (q0, q1), (k0, k1), (v0, v1)

    def x_rows(t):
        return pl.ds(_aligned(((t % NB) // 2) * BM, BM), BM)

    def x_copy(b, slot):
        return pltpu.make_async_copy(x_hbm.at[pl.ds(_aligned(b * BM, BM), BM), :], xs[slot].at[x_rows(b), :], xsem.at[b])

    def out_copy(b, slot):
        return pltpu.make_async_copy(xs[slot].at[x_rows(b), :], out_hbm.at[pl.ds(_aligned(b * BM, BM), BM), :], xsem.at[b])

    def wq_copy(p, i):
        r = pl.ds(_aligned(i * KP, KP), KP)
        return pltpu.make_async_copy((wqa_hbm, wqb_hbm)[p].at[r, :], wq_raw.at[p, r, :], wsem.at[p * (NK + 1) + i])

    def wo_copy(p):
        return pltpu.make_async_copy((woa_hbm, wob_hbm)[p], wo_raw.at[p], wsem.at[p * (NK + 1) + NK])

    x_copy(0, 0).start()
    wq_copy(0, 0).start()
    wq_copy(0, 1).start()
    x_copy(0, 0).wait()

    odd[...] = pltpu.bitcast(xs0[:16, :LANES], I32) | 3
    word = odd[0, 0]
    zeros = ((word & 1) - 1, (word & 2) - 2)
    site = [0]
    issued = []

    def fresh(v, m):
        site[0] += 1
        return pl.multiple_of(v + zeros[0] * (site[0] * m), m)

    def after(w, tok, r, c):
        if tok is None:
            return w
        head = jnp.where(odd[...] != 0, w[r:r + 8, c:c + LANES], tok)
        mid = [p for p in (w[r:r + 8, :c], head, w[r:r + 8, c + LANES:]) if p.shape[1]]
        out = [p for p in (w[:r], jnp.concatenate(mid, axis=1), w[r + 8:]) if p.shape[0]]
        return jnp.concatenate(out, axis=0)

    def not_before(v, back):
        if not issued:
            return v
        tok = pltpu.bitcast(issued[max(len(issued) - back, 0)], v.dtype)
        keep = odd[...] != 0
        return jnp.concatenate([jnp.where(keep, v[:, c:c + LANES], tok) for c in range(0, v.shape[1], LANES)], axis=1)

    def weave(matmuls, side, lo=0):
        n = 2 * len(matmuls)
        plan = [[] for _ in range(n)]
        for gen, count, lead, start in side:
            for i in range(count):
                plan[start + i * (n - start) // count].append((gen, lead))
        due = [[] for _ in range(n + max(B_LEAD, N_LEAD))]
        for i, f in enumerate(matmuls):
            for pt in (2 * i, 2 * i + 1):
                for gen, lead in plan[pt]:
                    tok = next(gen)
                    if lead is not None:
                        due[pt + lead].append(tok)
            issued.append(f([functools.reduce(jnp.bitwise_or, d) if d else None for d in due[2 * i:2 * i + 2]]))

    def prep_wq(p, g, ks):
        r = lax.broadcasted_iota(I32, (LANES, LANES), 0)
        n = lax.broadcasted_iota(I32, (LANES, LANES), 1)
        sel = [(n == (r % 4) * DH + 2 * (r // 8) + ((r // 4) % 2 ^ f)).astype(BF16) for f in range(2)]
        low = lax.broadcasted_iota(I32, (8, KP), 0) < 4
        y = [lax.dot_general(sel[i % 2], wq_raw[p, ks, g * GW + i * LANES:g * GW + (i + 1) * LANES], _NT,
                             preferred_element_type=F32) for i in range(4)]
        base = (g // 2) * (D // 2) + (g % 2) * 8
        for u in range(DH // 2):
            t = [v[8 * u:8 * u + 8] for v in y]
            even = [jnp.where(low, t[i], t[i + 1]) for i in (0, 2)]
            uneven = [pltpu.roll(jnp.where(low, t[i + 1], t[i]), 4, 0) for i in (0, 2)]
            for e, v in enumerate((even, uneven)):
                row = base + (2 * u + e) * (H // 2)
                wqT[p, row:row + 8, ks] = _pack(jnp.concatenate(v, axis=0))

    def prep_wo(p, j):
        cols = pl.ds(_aligned(j * LANES, LANES), LANES)
        for h in range(H):
            tbuf[h * PADH:h * PADH + DH, :] = wo_raw[p, h * DH:(h + 1) * DH, cols].astype(F32)
            if (h + 1) % (H // 2) == 0:
                yield None
        for d in range(DH):
            wop[p, d * (H // 2):(d + 1) * (H // 2), cols] = _pack(tbuf[pl.ds(d, H, stride=PADH), :])
            if (d + 1) % (DH // 2) == 0:
                yield None

    def weights_of(t):
        return (t // NB) % 2

    def norm_chunk(t, slot, c):
        r = pl.ds(_aligned(((t % NB) // 2) * BM + c * CH, CH), CH)
        xv = _unpack(not_before(pltpu.bitcast(xs[slot][r, :], U32), N_BACK)).astype(F32)
        xc = xv - jnp.mean(xv, axis=-1, keepdims=True)
        var = jnp.mean(xc * xc, axis=-1, keepdims=True)
        pk = _pack(xc * lax.rsqrt(var + 1e-5))
        xn[slot][pl.ds(_aligned(c * (CH // 2), CH // 2), CH // 2), :] = pk
        return pk

    def stage_n(t, slot):
        for c in range(BM // CH):
            yield _token([norm_chunk(t, slot, c)])

    def norm_block(t):
        @pl.loop(0, BM // CH)
        def _(c):
            norm_chunk(t, t % 2, c)

    def qkv_dst(slot, c):
        sec, j = divmod(c, NJ)
        r0 = 0 if sec == 0 else HALO
        return (qb, kb, vb)[sec][slot], (j, slice(r0, r0 + BM), slice(None))

    def stage_a(t, slot):
        def job(c, toks):
            wt = wqT[weights_of(t), pl.ds(fresh(c * LANES // 2, LANES // 2), LANES // 2), :]
            wt = after(after(wt, toks[0], 0, 0), toks[1], 0, D // 2)
            y = lax.dot_general(_unpack(xn[slot][...]), _unpack(wt), _NT, preferred_element_type=F32)
            dst, idx = qkv_dst(slot, c)
            dst[idx] = y
            return y[:8]
        return [functools.partial(job, c) for c in range(3 * NJ)]

    def halo(t, slot):
        first = (t % NB) == 0
        for bufs in (kb, vb):
            for j in range(NJ):
                row0 = jnp.broadcast_to(bufs[slot][j, HALO:HALO + 1, :], (HALO, LANES))
                if first is True:
                    bufs[slot][j, :HALO, :] = row0
                elif first is False:
                    bufs[slot][j, :HALO, :] = bufs[1 - slot][j, BM:BM + HALO, :]
                else:
                    bufs[slot][j, :HALO, :] = jnp.where(first, row0, bufs[1 - slot][j, BM:BM + HALO, :])

    def stage_b(t, slot):
        for c in range(BM // CH):
            probs = []
            for g in range(CH // 8):
                r0 = c * CH + 8 * g
                q = [not_before(qb[slot][j, r0:r0 + 8, :], B_BACK) for j in range(NJ)]
                logits = []
                for w in range(W):
                    rows = pl.ds(zeros[g % 2] + HALO + r0 - DIL * w, 8)
                    acc = q[0] * kb[slot][0, rows, :]
                    for j in range(1, NJ):
                        acc = acc + q[j] * kb[slot][j, rows, :]
                    acc = acc + pltpu.roll(acc, 2 * H, 1)
                    acc = acc + pltpu.roll(acc, H, 1)
                    if r0 < DIL * w:
                        pos = (t % NB) * BM + r0 + lax.broadcasted_iota(I32, (8, LANES), 0)
                        acc = jnp.where(pos >= DIL * w, acc, -1e9 / SCALE)
                    logits.append(acc)
                    if (w + 1) % W_PER_PHASE == 0 and w + 1 < W:
                        yield _token(logits[-W_PER_PHASE:])
                top = functools.reduce(jnp.maximum, logits)
                e = [jnp.exp2((lg - top) * (SCALE * LOG2E)) for lg in logits]
                inv = 1.0 / functools.reduce(jnp.add, e)
                probs.append([ew * inv for ew in e])
                yield _token([inv])
            p = [jnp.concatenate([pg[w] for pg in probs], axis=0) for w in range(W)]
            outs = []
            for j in range(NJ):
                acc = None
                for w in range(W):
                    a0 = zeros[c % 2] + HALO + c * CH - DIL * w
                    vv = jnp.concatenate([vb[slot][j, pl.ds(a0 + u, 8), :] for u in range(0, CH, 8)], axis=0)
                    acc = p[w] * vv if acc is None else acc + p[w] * vv
                pk = _pack(acc)
                ob[slot][c * (CH // 2):(c + 1) * (CH // 2), j * LANES:(j + 1) * LANES] = pk
                outs.append(pk)
                if (j + 1) % J_PER_PHASE == 0:
                    yield _token(outs[-J_PER_PHASE:])

    def stage_c(t, slot):
        def job(c, toks):
            cols = slice(c * LANES, (c + 1) * LANES)
            wt = wop[weights_of(t), :, pl.ds(fresh(c * LANES, LANES), LANES)]
            wt = after(after(wt, toks[0], 0, 0), toks[1], D // 4, 0)
            y = jnp.dot(_unpack(ob[slot][...]), _unpack(wt), preferred_element_type=F32)
            xs[slot][x_rows(t), cols] = (xs[slot][x_rows(t), cols].astype(F32) + y).astype(BF16)
            return y[:8]
        return [functools.partial(job, c) for c in range(NJ)]

    def step(t, slot):
        halo(t, slot)
        weave(stage_c(t - 1, 1 - slot) + stage_a(t + 1, 1 - slot),
              [(stage_b(t, slot), B_PHASES, B_LEAD, 0), (stage_n(t + 2, slot), BM // CH, N_LEAD, 0)])

    norm_block(0)

    @pl.loop(0, NK)
    def _(i):
        wq_copy(0, i).wait()

        @pl.when(i + 2 < NK)
        def _():
            wq_copy(0, i + 2).start()

        @pl.when(i + 2 == NK)
        def _():
            x_copy(1, 1).start()
            x_copy(2, 0).start()
            wo_copy(0).start()

        ks = pl.ds(pl.multiple_of(i * KP, KP), KP)

        def partial_qkv(sec):
            for c in range(sec * NJ, (sec + 1) * NJ):
                y = lax.dot_general(_unpack(xn0[:, ks]), _unpack(wqT[0, c * LANES // 2:(c + 1) * LANES // 2, ks]),
                                    _NT, preferred_element_type=F32)
                dst, idx = qkv_dst(0, c)
                dst[idx] = jnp.where(i == 0, y, dst[idx] + y)

        for g in range(3 * D // GW):
            prep_wq(0, g, ks)
            if g == 3:
                partial_qkv(0)
        partial_qkv(1)
        partial_qkv(2)

    def prep_wo_a():
        wo_copy(0).wait()
        for b in range(3, NB):
            x_copy(b, b % 2).start()
        for j in range(NJ):
            yield from prep_wo(0, j)

    halo(0, 0)
    x_copy(1, 1).wait()
    norm_block(1)
    x_copy(2, 0).wait()
    weave(stage_a(1, 1), [(stage_b(0, 0), B_PHASES, B_LEAD, 0), (stage_n(2, 0), BM // CH, N_LEAD, 0),
                          (prep_wo_a(), NJ * WO_PHASES, None, 2 * NJ)])

    @pl.loop(0, T // 2 - 1)
    def _(i):
        @pl.when(2 * i + 3 < NB)
        def _():
            x_copy(2 * i + 3, 1).wait()

        @pl.when(2 * i + 4 < NB)
        def _():
            x_copy(2 * i + 4, 0).wait()

        @pl.when(i == 1)
        def _():
            for s in range(NK):
                wq_copy(1, s).start()
            wo_copy(1).start()

        @pl.when(i == NB // 2 - 1)
        def _():
            for s in range(NK):
                wq_copy(1, s).wait()
            wo_copy(1).wait()

            @pl.loop(0, NK)
            def _(s):
                for g in range(3 * D // GW):
                    prep_wq(1, g, pl.ds(pl.multiple_of(s * KP, KP), KP))
                for u in range(NJ // NK):
                    _drain(prep_wo(1, s * (NJ // NK) + u))

        issued.clear()
        step(2 * i + 1, 1)
        step(2 * i + 2, 0)

        @pl.when(2 * i >= T - NB)
        def _():
            out_copy(2 * i - (T - NB), 0).start()
            out_copy(2 * i + 1 - (T - NB), 1).start()

    issued.clear()
    halo(T - 1, 1)
    weave(stage_c(T - 2, 0), [(stage_b(T - 1, 1), B_PHASES, B_LEAD, 0)])
    out_copy(NB - 2, 0).start()
    weave(stage_c(T - 1, 1), [])
    out_copy(NB - 1, 1).start()
    for b in range(NB):
        out_copy(b, b % 2).wait()


@jax.jit
def pallas_interleave_layers__sliding_local_dilated__sliding_local_dilated__prompt_kernel(
    A_x: jax.Array,
    A_wqkv: jax.Array,
    A_wo: jax.Array,
    B_x: jax.Array,
    B_wqkv: jax.Array,
    B_wo: jax.Array,
):
    del B_x
    any_spec = pl.BlockSpec(memory_space=pl.ANY)
    out = pl.pallas_call(
        _kernel,
        out_shape=jax.ShapeDtypeStruct((S, D), BF16),
        in_specs=[any_spec] * 5,
        out_specs=any_spec,
        scratch_shapes=(
            [pltpu.VMEM((S // 2, D), BF16)] * 2
            + [pltpu.VMEM((HB, D), U32)] * 4
            + [pltpu.VMEM((NJ, BM, LANES), F32)] * 2
            + [pltpu.VMEM((NJ, HALO + BM, LANES), F32)] * 4
            + [pltpu.VMEM((2, 3 * D // 2, D), U32),
               pltpu.VMEM((2, D // 2, D), U32),
               pltpu.VMEM((2, D, 3 * D), BF16),
               pltpu.VMEM((2, D, D), BF16),
               pltpu.VMEM((H * PADH, LANES), F32),
               pltpu.VMEM((8, LANES), I32),
               pltpu.SemaphoreType.DMA((NB,)),
               pltpu.SemaphoreType.DMA((2 * (NK + 1),))]),
        compiler_params=pltpu.CompilerParams(vmem_limit_bytes=96 * 2**20),
    )(A_x.reshape(S, D), A_wqkv, A_wo, B_wqkv, B_wo)
    return out.reshape(A_x.shape)
```

```python
import functools

import jax
import jax.numpy as jnp
from jax import lax
from jax.experimental import pallas as pl
from jax.experimental.pallas import tpu as pltpu

S, D, H, W, DIL = 2048, 1024, 32, 8, 2
DH = D // H
N_LAYERS = 4
LANES = 128
NJ = D // LANES
BM = 128
HB = BM // 2
NB = S // BM
T = N_LAYERS * NB
HALO = 16
CH = 16
KP = 256
NK = D // KP
GW = 4 * LANES
PADH = DH + 1
SCALE = DH ** -0.5
LOG2E = 1.4426950408889634
F32, BF16, U32, I32 = jnp.float32, jnp.bfloat16, jnp.uint32, jnp.int32

B_LEAD, B_BACK = 5, 3
N_LEAD, N_BACK = 6, 2
W_PER_PHASE, J_PER_PHASE = 4, 2
B_PHASES = (BM // CH) * ((CH // 8) * (W // W_PER_PHASE) + NJ // J_PER_PHASE)
WO_PHASES = 4
A_AHEAD, C_STRIDE = (4, 0), 4

_NT = (((1,), (1,)), ((), ()))


def _pack(v):
    return pltpu.bitcast(v.astype(BF16), U32)


def _unpack(v):
    return pltpu.bitcast(v, BF16)


def _token(vals):
    parts = []
    for v in vals:
        v = v if v.dtype == U32 else pltpu.bitcast(v, U32)
        parts += [v[r:r + 8, c:c + LANES] for r in range(0, v.shape[0], 8) for c in range(0, v.shape[1], LANES)]
    return functools.reduce(jnp.bitwise_or, parts)


def _aligned(v, m):
    return v if isinstance(v, int) else pl.multiple_of(v, m)


def _drain(gen):
    for _ in gen:
        pass


def _kernel(x_hbm, wqa_hbm, woa_hbm, wqb_hbm, wob_hbm, out_hbm,
            xs0, xs1, xn0, xn1, ob0, ob1, q0, q1, k0, k1, v0, v1,
            wqT, wop, wq_raw, wo_raw, tbuf, pick, odd, xsem, wsem):
    xs, xn, ob, qb, kb, vb = (xs0, xs1), (xn0, xn1), (ob0, ob1), (q0, q1), (k0, k1), (v0, v1)

    def x_rows(t):
        return pl.ds(_aligned(((t % NB) // 2) * BM, BM), BM)

    def x_copy(b, slot):
        return pltpu.make_async_copy(x_hbm.at[pl.ds(_aligned(b * BM, BM), BM), :], xs[slot].at[x_rows(b), :], xsem.at[b])

    def out_copy(b, slot):
        return pltpu.make_async_copy(xs[slot].at[x_rows(b), :], out_hbm.at[pl.ds(_aligned(b * BM, BM), BM), :], xsem.at[b])

    def wq_copy(p, i):
        r = pl.ds(_aligned(i * KP, KP), KP)
        return pltpu.make_async_copy((wqa_hbm, wqb_hbm)[p].at[r, :], wq_raw.at[p, r, :], wsem.at[p * (NK + 1) + i])

    def wo_copy(p):
        return pltpu.make_async_copy((woa_hbm, wob_hbm)[p], wo_raw.at[p], wsem.at[p * (NK + 1) + NK])

    x_copy(0, 0).start()
    x_copy(1, 1).start()
    wq_copy(0, 0).start()
    x_copy(0, 0).wait()

    odd[...] = pltpu.bitcast(xs0[:16, :LANES], I32) | 3
    word = odd[0, 0]
    zeros = ((word & 1) - 1, (word & 2) - 2)
    site = [0]
    issued = []

    def fresh(v, m):
        site[0] += 1
        return pl.multiple_of(v + zeros[0] * (site[0] * m), m)

    def after(w, tok, r, c):
        if tok is None:
            return w
        head = jnp.where(odd[...] != 0, w[r:r + 8, c:c + LANES], tok)
        mid = [p for p in (w[r:r + 8, :c], head, w[r:r + 8, c + LANES:]) if p.shape[1]]
        out = [p for p in (w[:r], jnp.concatenate(mid, axis=1), w[r + 8:]) if p.shape[0]]
        return jnp.concatenate(out, axis=0)

    def not_before(v, back):
        if not issued:
            return v
        tok = pltpu.bitcast(issued[max(len(issued) - back, 0)], v.dtype)
        return jnp.where(odd[...] != 0, v, tok)

    def weave(matmuls, side, carried=()):
        n = 2 * len(matmuls)
        plan = [[] for _ in range(n)]
        for gen, count, lead, start in side:
            for i in range(count):
                plan[start + i * (n - start) // count].append((gen, lead))
        due = [[] for _ in range(n + max(B_LEAD, N_LEAD))]
        for pt, toks in enumerate(carried):
            due[pt] += toks
        for i, f in enumerate(matmuls):
            for pt in (2 * i, 2 * i + 1):
                for gen, lead in plan[pt]:
                    tok = next(gen)
                    if lead is not None:
                        due[pt + lead].append(tok)
            issued.append(f([functools.reduce(jnp.bitwise_or, d) if d else None for d in due[2 * i:2 * i + 2]]))
        return due[n:]

    row = lax.broadcasted_iota(I32, (LANES, LANES), 0)
    col = lax.broadcasted_iota(I32, (LANES, LANES), 1)
    for f in range(2):
        pick[f] = _pack((col == (row % 4) * DH + 2 * (row // 8) + ((row // 4) % 2 ^ f)).astype(F32))

    def prep_wq(p, g, ks):
        sel = [_unpack(pick[f]) for f in range(2)]
        low = lax.broadcasted_iota(I32, (8, KP), 0) < 4
        y = [lax.dot_general(sel[i % 2], wq_raw[p, ks, g * GW + i * LANES:g * GW + (i + 1) * LANES], _NT,
                             preferred_element_type=F32) for i in range(4)]
        base = (g // 2) * (D // 2) + (g % 2) * 8
        for u in range(DH // 2):
            t = [v[8 * u:8 * u + 8] for v in y]
            even = [jnp.where(low, t[i], t[i + 1]) for i in (0, 2)]
            uneven = [pltpu.roll(jnp.where(low, t[i + 1], t[i]), 4, 0) for i in (0, 2)]
            for e, v in enumerate((even, uneven)):
                r = base + (2 * u + e) * (H // 2)
                wqT[p, r:r + 8, ks] = _pack(jnp.concatenate(v, axis=0))

    def prep_wo(p, j):
        cols = pl.ds(_aligned(j * LANES, LANES), LANES)
        for h in range(H):
            tbuf[h * PADH:h * PADH + DH, :] = wo_raw[p, h * DH:(h + 1) * DH, cols].astype(F32)
            if (h + 1) % (H // 2) == 0:
                yield None
        for d in range(DH):
            wop[p, d * (H // 2):(d + 1) * (H // 2), cols] = _pack(tbuf[pl.ds(d, H, stride=PADH), :])
            if (d + 1) % (DH // 2) == 0:
                yield None

    def weights_of(t):
        return (t // NB) % 2

    def stage_n(t, slot):
        for c in range(BM // CH):
            r = pl.ds(_aligned(((t % NB) // 2) * BM + c * CH, CH), CH)
            words = pltpu.bitcast(xs[slot][r, :], U32)
            words = jnp.concatenate([not_before(words[:, :LANES], N_BACK), words[:, LANES:]], axis=1)
            xv = _unpack(words).astype(F32)
            xc = xv - jnp.mean(xv, axis=-1, keepdims=True)
            var = jnp.mean(xc * xc, axis=-1, keepdims=True)
            pk = _pack(xc * lax.rsqrt(var + 1e-5))
            xn[slot][c * (CH // 2):(c + 1) * (CH // 2), :] = pk
            yield _token([pk])

    def qkv_dst(slot, c):
        sec, j = divmod(c, NJ)
        r0 = 0 if sec == 0 else HALO
        return (qb, kb, vb)[sec][slot], (j, slice(r0, r0 + BM), slice(None))

    def stage_a(t, slot):
        def job(c, toks):
            wt = wqT[weights_of(t), pl.ds(fresh(c * LANES // 2, LANES // 2), LANES // 2), :]
            wt = after(after(wt, toks[0], 0, 0), toks[1], 0, D // 2)
            y = lax.dot_general(_unpack(xn[slot][...]), _unpack(wt), _NT, preferred_element_type=F32)
            dst, idx = qkv_dst(slot, c)
            dst[idx] = y
            return y[:8]
        return [functools.partial(job, c) for c in range(3 * NJ)]

    def halo(t, slot):
        first = (t % NB) == 0
        for bufs in (kb, vb):
            for j in range(NJ):
                row0 = jnp.broadcast_to(bufs[slot][j, HALO:HALO + 1, :], (HALO, LANES))
                if first is True:
                    bufs[slot][j, :HALO, :] = row0
                elif first is False:
                    bufs[slot][j, :HALO, :] = bufs[1 - slot][j, BM:BM + HALO, :]
                else:
                    bufs[slot][j, :HALO, :] = jnp.where(first, row0, bufs[1 - slot][j, BM:BM + HALO, :])

    def stage_b(t, slot):
        for c in range(BM // CH):
            probs = []
            for g in range(CH // 8):
                r0 = c * CH + 8 * g
                q = [qb[slot][j, r0:r0 + 8, :] for j in range(NJ)]
                q = [not_before(v, B_BACK) for v in q]
                logits = []
                for w in range(W):
                    rows = pl.ds(zeros[g % 2] + HALO + r0 - DIL * w, 8)
                    acc = functools.reduce(jnp.add, [q[j] * kb[slot][j, rows, :] for j in range(NJ)])
                    acc = acc + pltpu.roll(acc, 2 * H, 1)
                    acc = acc + pltpu.roll(acc, H, 1)
                    if r0 < DIL * w:
                        pos = (t % NB) * BM + r0 + lax.broadcasted_iota(I32, (8, LANES), 0)
                        acc = jnp.where(pos >= DIL * w, acc, -1e9 / SCALE)
                    logits.append(acc)
                    if (w + 1) % W_PER_PHASE == 0 and w + 1 < W:
                        yield _token(logits[-W_PER_PHASE:])
                top = functools.reduce(jnp.maximum, logits)
                e = [jnp.exp2((lg - top) * (SCALE * LOG2E)) for lg in logits]
                inv = 1.0 / functools.reduce(jnp.add, e)
                probs.append(e + [inv])
                yield _token([inv])
            *e, inv = [jnp.concatenate(groups, axis=0) for groups in zip(*probs)]
            outs = []
            for j in range(NJ):
                terms = []
                for w in range(W):
                    a0 = zeros[c % 2] + HALO + c * CH - DIL * w
                    vv = jnp.concatenate([vb[slot][j, pl.ds(a0 + u, 8), :] for u in range(0, CH, 8)], axis=0)
                    terms.append(e[w] * vv)
                pk = _pack(functools.reduce(jnp.add, terms) * inv)
                ob[slot][c * (CH // 2):(c + 1) * (CH // 2), j * LANES:(j + 1) * LANES] = pk
                outs.append(pk)
                if (j + 1) % J_PER_PHASE == 0:
                    yield _token(outs[-J_PER_PHASE:])

    def stage_c(t, slot):
        def job(c, toks):
            cols = slice(c * LANES, (c + 1) * LANES)
            wt = wop[weights_of(t), :, pl.ds(fresh(c * LANES, LANES), LANES)]
            wt = after(after(wt, toks[0], 0, 0), toks[1], D // 4, 0)
            y = jnp.dot(_unpack(ob[slot][...]), _unpack(wt), preferred_element_type=F32)
            xs[slot][x_rows(t), cols] = (xs[slot][x_rows(t), cols].astype(F32) + y).astype(BF16)
            return y[:8]
        return [functools.partial(job, c) for c in range(NJ)]

    def step(t, slot, carried=()):
        halo(t, slot)
        qkv = stage_a(t + 1, 1 - slot)
        order, rest = qkv[:A_AHEAD[slot]], qkv[A_AHEAD[slot]:]
        for job in stage_c(t - 1, 1 - slot):
            order += [job] + rest[:C_STRIDE - 1]
            rest = rest[C_STRIDE - 1:]
        return weave(order + rest, [(stage_b(t, slot), B_PHASES, B_LEAD, 0),
                                    (stage_n(t + 2, slot), BM // CH, N_LEAD, 0)], carried)

    _drain(stage_n(0, 0))
    x_copy(1, 1).wait()
    _drain(stage_n(1, 1))

    @pl.loop(0, NK)
    def _(i):
        wq_copy(0, i).wait()

        @pl.when(i + 1 < NK)
        def _():
            wq_copy(0, i + 1).start()

        @pl.when(i + 1 == NK)
        def _():
            x_copy(2, 0).start()
            wo_copy(0).start()

        ks = pl.ds(pl.multiple_of(i * KP, KP), KP)

        def partial_qkv(sec):
            for c in range(sec * NJ, (sec + 1) * NJ):
                y = lax.dot_general(_unpack(xn0[:, ks]), _unpack(wqT[0, c * LANES // 2:(c + 1) * LANES // 2, ks]),
                                    _NT, preferred_element_type=F32)
                dst, idx = qkv_dst(0, c)
                dst[idx] = jnp.where(i == 0, y, dst[idx] + y)

        for g in range(3 * D // GW):
            prep_wq(0, g, ks)
            if g == 3:
                partial_qkv(0)
        partial_qkv(1)
        partial_qkv(2)

    def prep_wo_a():
        wo_copy(0).wait()
        for b in range(3, NB):
            x_copy(b, b % 2).start()
        for j in range(NJ):
            yield from prep_wo(0, j)

    halo(0, 0)
    x_copy(2, 0).wait()
    weave(stage_a(1, 1), [(stage_b(0, 0), B_PHASES, B_LEAD, 0), (stage_n(2, 0), BM // CH, N_LEAD, 0),
                          (prep_wo_a(), NJ * WO_PHASES, None, 2 * NJ)])

    @pl.loop(0, T // 2 - 1)
    def _(i):
        @pl.when(i < NB // 2)
        def _():
            @pl.when(2 * i + 3 < NB)
            def _():
                x_copy(2 * i + 3, 1).wait()

            @pl.when(2 * i + 4 < NB)
            def _():
                x_copy(2 * i + 4, 0).wait()

            @pl.when(i == 1)
            def _():
                for s in range(NK):
                    wq_copy(1, s).start()
                wo_copy(1).start()

            @pl.when(i == NB // 2 - 1)
            def _():
                for s in range(NK):
                    wq_copy(1, s).wait()
                wo_copy(1).wait()

                @pl.loop(0, NK)
                def _(s):
                    for g in range(3 * D // GW):
                        prep_wq(1, g, pl.ds(pl.multiple_of(s * KP, KP), KP))
                    for u in range(NJ // NK):
                        _drain(prep_wo(1, s * (NJ // NK) + u))

        issued.clear()
        step(2 * i + 2, 0, step(2 * i + 1, 1))

        @pl.when(2 * i >= T - NB)
        def _():
            out_copy(2 * i - (T - NB), 0).start()
            out_copy(2 * i + 1 - (T - NB), 1).start()

    issued.clear()
    halo(T - 1, 1)
    weave(stage_c(T - 2, 0), [(stage_b(T - 1, 1), B_PHASES, B_LEAD, 0)])
    out_copy(NB - 2, 0).start()
    weave(stage_c(T - 1, 1), [])
    out_copy(NB - 1, 1).start()
    for b in range(NB):
        out_copy(b, b % 2).wait()


@jax.jit
def pallas_interleave_layers__sliding_local_dilated__sliding_local_dilated__prompt_kernel(
    A_x: jax.Array,
    A_wqkv: jax.Array,
    A_wo: jax.Array,
    B_x: jax.Array,
    B_wqkv: jax.Array,
    B_wo: jax.Array,
):
    del B_x
    any_spec = pl.BlockSpec(memory_space=pl.ANY)
    out = pl.pallas_call(
        _kernel,
        out_shape=jax.ShapeDtypeStruct((S, D), BF16),
        in_specs=[any_spec] * 5,
        out_specs=any_spec,
        scratch_shapes=(
            [pltpu.VMEM((S // 2, D), BF16)] * 2
            + [pltpu.VMEM((HB, D), U32)] * 4
            + [pltpu.VMEM((NJ, BM, LANES), F32)] * 2
            + [pltpu.VMEM((NJ, HALO + BM, LANES), F32)] * 4
            + [pltpu.VMEM((2, 3 * D // 2, D), U32),
               pltpu.VMEM((2, D // 2, D), U32),
               pltpu.VMEM((2, D, 3 * D), BF16),
               pltpu.VMEM((2, D, D), BF16),
               pltpu.VMEM((H * PADH + DH, LANES), F32),
               pltpu.VMEM((2, LANES // 2, LANES), U32),
               pltpu.VMEM((8, LANES), I32),
               pltpu.SemaphoreType.DMA((NB,)),
               pltpu.SemaphoreType.DMA((2 * (NK + 1),))]),
        compiler_params=pltpu.CompilerParams(vmem_limit_bytes=96 * 2**20),
    )(A_x.reshape(S, D), A_wqkv, A_wo, B_wqkv, B_wo)
    return out.reshape(A_x.shape)
```
